```python
import jax
import jax.numpy as jnp

def _softmax(x, axis=-1):
    return jax.nn.softmax(x, axis=axis)
def _gelu(x):
    return jax.nn.gelu(x, approximate=True)
def _silu(x):
    return jax.nn.silu(x)
def _sigmoid(x):
    return jax.nn.sigmoid(x)
def _layernorm(x, axis=-1, eps=1e-5):
    m = jnp.mean(x, axis=axis, keepdims=True)
    v = jnp.var(x, axis=axis, keepdims=True)
    return (x - m) / jnp.sqrt(v + eps)
def _scatter_add(tgt, idx, src, axis=0):
    return tgt.at[idx].add(src)
def _segment_sum(src, seg, n):
    return jax.ops.segment_sum(src, seg, n)
class _Rng:
    def __init__(self, key):
        self._k = key
    def _next(self):
        self._k, sub = jax.random.split(self._k)
        return sub
    def normal(self, shape):
        return jax.random.normal(self._next(), shape, dtype=jnp.bfloat16)
    def randint(self, lo, hi, shape):
        return jax.random.randint(self._next(), shape, lo, hi, dtype=jnp.int32)
    def uniform(self, shape, lo=0.0, hi=1.0):
        return jax.random.uniform(self._next(), shape, jnp.bfloat16, lo, hi)
    def permutation(self, n):
        return jax.random.permutation(self._next(), n)


kernel_name = 'gated_mix__sliding_block_cached__glu_gated_swiglu__decode'

def setup_inputs():
    _rng = _Rng(jax.random.key(int.from_bytes(__import__("os").urandom(4), "little")))
    _w = (lambda a: (lambda t: t.astype(jnp.bfloat16) if jnp.issubdtype(t.dtype, jnp.floating) else t)(jnp.asarray(a)))
    def _A_setup():
        B, Sq, D = 1, 1, 640
        Hq, Hkv, Sk, Dh = 32, 32, 32768, 192
        assert Hq % Hkv == 0, (Hq, Hkv)
        return {
            "x": _w((lambda *s: _rng.normal(s) * 0.05)(B, Sq, D)),
            "k_cache": _w((lambda *s: _rng.normal(s) * 0.05)(B, Hkv, Sk, Dh)),
            "v_cache": _w((lambda *s: _rng.normal(s) * 0.05)(B, Hkv, Sk, Dh)),
            "wq": _w((lambda *s: _rng.normal(s) * 0.05)(D, Hq * Dh) * (D ** -0.5)),
            "wo": _w((lambda *s: _rng.normal(s) * 0.05)(Hq * Dh, D) * ((Hq * Dh) ** -0.5)),
        }
    _A_in = _A_setup()

    def _B_setup():
        B, S, D, F = 1, 1, 640, 1536
        return {
            "x": _w((lambda *s: _rng.normal(s) * 0.05)(B, S, D)),
            "w1": _w((lambda *s: _rng.normal(s) * 0.05)(D, F) * (2.0 / D) ** 0.5),
            "w3": _w((lambda *s: _rng.normal(s) * 0.05)(D, F) * (2.0 / D) ** 0.5),
            "w2": _w((lambda *s: _rng.normal(s) * 0.05)(F, D) * (2.0 / F) ** 0.5),
        }
    _B_in = _B_setup()

    return {
        "A_x": _A_in["x"],
        "A_k_cache": _A_in["k_cache"],
        "A_v_cache": _A_in["v_cache"],
        "A_wq": _A_in["wq"],
        "A_wo": _A_in["wo"],
        "B_x": _B_in["x"],
        "B_w1": _B_in["w1"],
        "B_w3": _B_in["w3"],
        "B_w2": _B_in["w2"],
        "gate_w": _w((lambda *s: _rng.normal(s) * 0.05)(640)),
    }

def reference(A_x, A_k_cache, A_v_cache, A_wq, A_wo, B_x, B_w1, B_w3, B_w2, gate_w):
    def _A_ref(x, k_cache, v_cache, wq, wo):
        B, Sq, D = x.shape
        Hq, Dh = 32, 192
        Hkv, Sk = k_cache.shape[1], k_cache.shape[2]
        W = min(4096, max(256, Sk // 4))
        rep = Hq // Hkv
        q = (lambda x, *d: x.transpose(*d))((x @ wq).reshape(B, Sq, Hq, Dh), 0, 2, 1, 3)
        k = jnp.repeat(k_cache[:, :, Sk - W:, :], rep, axis=1)
        v = jnp.repeat(v_cache[:, :, Sk - W:, :], rep, axis=1)
        scores = jnp.einsum("bhqd,bhkd->bhqk", q, k) * (Dh ** -0.5)
        p = _softmax(scores, axis=-1)
        o = jnp.einsum("bhqk,bhkd->bhqd", p, v)
        return (lambda x, *d: x.transpose(*d))(o, 0, 2, 1, 3).reshape(B, Sq, Hq * Dh) @ wo

    def _B_ref(x, w1, w3, w2):
        gate = jnp.einsum("bsd,df->bsf", x, w1)
        up = jnp.einsum("bsd,df->bsf", x, w3)
        h = _silu(gate) * up
        out = jnp.einsum("bsf,fd->bsd", h, w2)
        return out

    x = A_x
    g = _sigmoid((x * gate_w).sum(-1, keepdims=True))
    a = _A_ref(x, A_k_cache, A_v_cache, A_wq, A_wo)
    b = _B_ref(x, B_w1, B_w3, B_w2)
    return g * a + (1 - g) * b
```

```python
import jax
import jax.numpy as jnp
from jax import lax
import jax.experimental.pallas as pl
import jax.experimental.pallas.tpu as pltpu

_NT = (((1,), (1,)), ((), ()))
_F32 = jnp.float32
_BF16 = jnp.bfloat16


def _tiles(w, n):
    R, C = w.shape
    return w.reshape(R // 8, 8, C // 128, 128).transpose(0, 2, 1, 3).reshape(n, -1, 128)


def _iota(shape, d):
    return lax.broadcasted_iota(jnp.int32, shape, d)


def make(SH=25, LATE=11, tail=(5, 4, 2, 1), sub=4, order="g", nocompute=False, nobc=True, tail_mode="a",
         wpat=((1, 3), (1, 3), (1, 3), (1, 2)), tail_late=None):
    def fn(A_x, A_k_cache, A_v_cache, A_wq, A_wo, B_x, B_w1, B_w3, B_w2, gate_w):
        B, Sq, D = A_x.shape
        _, H, SK, DH = A_k_cache.shape
        F = B_w1.shape[1]
        W = min(4096, max(256, SK // 4))
        scale = DH ** -0.5
        CW = 1024
        RUN = 64
        GR = 8 * DH
        NG, NQ, NU = H // 8, W // CW, GR // 128
        kT = jnp.swapaxes(A_k_cache, 2, 3).reshape(H * DH, SK)
        vT = jnp.swapaxes(A_v_cache, 2, 3).reshape(H * DH, SK)
        wq, wo = _tiles(A_wq, 15), _tiles(A_wo, 15)
        w1, w3 = _tiles(B_w1, 4), _tiles(B_w3, 4)
        w2 = _tiles(B_w2, F // 128)

        def kernel(x_ref, k_ref, v_ref, wq_ref, wo_ref, w1_ref, w3_ref, w2_ref, gw_ref, o_ref,
                   kv_b, wq_b, wo_b, w1_b, w3_b, w2_b, x_b, gw_b, xq_s, xf_s, q_s, s_s, p_s, o_s, h_s, hc_s, out_b, osem):

            def rows(buf, r0, n):
                per = buf.shape[1]
                out, r = [], r0
                while r < r0 + n:
                    m = min(r0 + n - r, per - r % per)
                    out.append((r - r0, m, buf.at[r // per, pl.ds(r % per, m)]))
                    r += m
                return out

            def tile_dot(lhs, buf, r0):
                acc = None
                for (o, m, ref) in rows(buf, r0, lhs.shape[1]):
                    p = jnp.dot(lhs[:, o:o + m], ref[...], preferred_element_type=_F32)
                    acc = p if acc is None else acc + p
                return acc

            def body(sem):
                nsem = sem.shape[0]
                steps = []
                groups = []

                def w_steps(big, big_b, small, small_b):
                    g = len(groups)
                    for u in range(big.shape[1] // RUN):
                        def run(src, dst, r, n):
                            idx = (pl.ds(r, n), pl.ds(u * RUN, RUN))
                            return (src.at[idx], dst.at[idx])
                        if u < small.shape[1] // RUN:
                            steps.append((g, [run(small, small_b, 0, 1)], [run(small, small_b, 1, 3)]))
                        r = 0
                        for (a, b) in wpat:
                            steps.append((g, [run(big, big_b, r, a)], [run(big, big_b, r + a, b)]))
                            r += a + b
                    groups.append([big_b, small_b])

                w_steps(wq_ref, wq_b, w1_ref, w1_b)
                steps[4][1].extend([(x_ref, x_b), (gw_ref, gw_b)])
                groups[0] += [x_b, gw_b]
                w_steps(wo_ref, wo_b, w3_ref, w3_b)

                if order == "g":
                    kv_order = [(m, g, c) for g in range(NG) for m in (0, 1) for c in range(NQ)]
                else:
                    kv_order = [(m, g, c) for m in (0, 1) for c in range(NQ) for g in range(NG)]
                for n, (m, g, c) in enumerate(kv_order):
                    src, dst = (k_ref, v_ref)[m], kv_b.at[n % 3]
                    for r in range(0, GR, 32):
                        def run(r0, nr):
                            return (src.at[pl.ds(g * GR + r0, nr), pl.ds(SK - W + c * CW, CW)], dst.at[pl.ds(r0, nr)])
                        steps.append((len(groups), [run(r, 8)], [run(r + 8, 24)]))
                    groups.append([dst])
                T0 = len(groups)
                j0 = 0
                for t, nj in enumerate(tail):
                    def run(j, n, u, nu=1):
                        idx = (pl.ds(j, n), pl.ds(u * RUN, nu * RUN))
                        return (w2_ref.at[idx], w2_b.at[idx])
                    if nj >= 3:
                        for u in range(D // RUN):
                            steps.append((len(groups), [run(j0, 1, u)], [run(j0 + 1, nj - 1, u)]))
                    elif tail_mode == "a":
                        steps.append((len(groups), [], [run(j0, nj, 0, D // RUN)]))
                    elif tail_mode == "b":
                        for j in range(j0, j0 + nj):
                            for (u, n) in ((0, 4), (4, 3), (7, 3)):
                                steps.append((len(groups), [run(j, 1, u)], [run(j, 1, u + 1, n - 1)]))
                    groups.append([w2_b.at[pl.ds(j0, nj)]])
                    j0 += nj
                N = len(steps)
                end = {}
                for i, s in enumerate(steps):
                    end[s[0]] = i + 1

                def sem_of(g):
                    return sem.at[g % 2 if g < T0 else 2 + g - T0]

                pos = {"i": 0, "waited": -1}

                def advance(n):
                    while pos["i"] < min(n, N + SH):
                        i = pos["i"]
                        for (k, prio) in ((i - SH, 0), (i, 1)):
                            if 0 <= k < N:
                                g = steps[k][0]
                                assert g >= T0 or pos["waited"] >= g - 2
                                for (s_, d_) in steps[k][1 + prio]:
                                    pltpu.make_async_copy(s_, d_, sem_of(g)).start(priority=prio)
                        pos["i"] += 1

                def wait(g, late=LATE):
                    advance(end[g] + SH + late)
                    for ref in groups[g]:
                        pltpu.make_async_copy(ref, ref, sem_of(g)).wait()
                    pos["waited"] = g

                def run_tasks(tasks, until):
                    i0 = pos["i"]
                    for k, task in enumerate(tasks):
                        if not nocompute:
                            task()
                        advance(i0 + (until - i0) * (k + 1) // len(tasks))

                st = {}

                def prep():
                    x = x_b[0]
                    gw = gw_b[...].reshape(1, D).astype(_F32)
                    st["gate"] = jax.nn.sigmoid(jnp.sum(x.astype(_F32) * gw, axis=-1, keepdims=True))
                    xr = jnp.broadcast_to(x.astype(_F32), (D // 8, D))
                    xm = jnp.where(_iota((D // 8, D), 1) // 8 == _iota((D // 8, D), 0), xr, 0.0).astype(_BF16)
                    e = jnp.where(_iota((D, 128), 0) % 8 == _iota((D, 128), 1) % 8, 1.0, 0.0).astype(_BF16)
                    xq_s[...] = jnp.dot(xm, e, preferred_element_type=_F32)

                def prep_f(m):
                    def run():
                        l = _iota((1, 384), 1)
                        v = None
                        for i in range(4):
                            r = xq_s[4 * m + i:4 * m + i + 1, :]
                            r = jnp.concatenate([r, r, r], axis=1)
                            v = r if v is None else jnp.where(l >= 96 * i, r, v)
                        xf_s[m] = jnp.where((_iota((16, 384), 1) // 8) % 12 == _iota((16, 384), 0), v, 0.0).astype(_BF16)
                    return run

                def q_task(tr):
                    def run():
                        lhs = jnp.where(_iota((16, 128), 1) // 8 == _iota((16, 128), 0), xq_s[tr:tr + 1, :], 0.0).astype(_BF16)
                        for b in range(3):
                            p = tile_dot(lhs, wq_b, tr * 384 + b * 128)
                            st["q", b] = p if tr == 0 else st["q", b] + p
                    return run

                def head_mask(j):
                    d = _iota((8, 128), 1) + (j % NU) * 128 - _iota((8, 128), 0) * DH
                    return (d >= 0) & (d < DH)

                def q_spread(b):
                    def run():
                        for i in range(16):
                            j = 16 * b + i
                            q_s[j] = jnp.where(head_mask(j), st["q", b][i:i + 1, :], 0.0).astype(_BF16)
                    return run

                def f_task(name, buf, m):
                    def run():
                        p = tile_dot(xf_s[m], buf, m * 384)
                        st[name] = p if m == 0 else st[name] + p
                    return run

                def spread5(v):
                    l = _iota((128, D), 1)
                    e = jnp.where(_iota((128, D), 0) == 8 * (l // 40) + l % 8, 1.0, 0.0).astype(_BF16)
                    return jnp.dot(v, e, preferred_element_type=_F32)

                def diag5(row):
                    return jnp.where((_iota((8, D), 1) // 8) % 5 == _iota((8, D), 0), row, 0.0).astype(_BF16)

                def glu():
                    g_, u_ = st["g"], st["u"]
                    h = (g_ * jax.nn.sigmoid(g_) * u_).astype(_BF16)
                    h5 = spread5(h)
                    for j in range(F // 128):
                        h_s[j] = diag5(h5[j:j + 1, :])
                    hl = h[F // 128 - 1:F // 128, :].astype(_F32)
                    hc_s[...] = jnp.transpose(jnp.broadcast_to(hl, (128, 128)))

                wait(0)
                run_tasks([prep] + [prep_f(m) for m in range(D // 32)] + [q_task(t) for t in range(D // 8)]
                          + [q_spread(b) for b in range(3)]
                          + [f_task("g", w1_b, m) for m in range(D // 32)], end[1] + SH + LATE)
                wait(1)
                run_tasks([f_task("u", w3_b, m) for m in range(D // 32)] + [glu], end[2] + SH + LATE)

                cw = CW // sub

                def qk_task(buf, g, c, u, part):
                    def run():
                        p = jnp.dot(q_s[g * NU + u], buf[u * 128:(u + 1) * 128, part * cw:(part + 1) * cw],
                                    preferred_element_type=_F32)
                        st["s", part] = p if u == 0 else st["s", part] + p
                        if u == NU - 1:
                            n0 = c * CW + part * cw
                            s_s[g, :, n0:n0 + cw] = st["s", part] * scale
                    return run

                def softmax(g):
                    def run():
                        s = s_s[g]
                        e = jnp.exp(s - jnp.max(s, axis=-1, keepdims=True))
                        p_s[g] = (e * (1.0 / jnp.sum(e, axis=-1, keepdims=True))).astype(_BF16)
                    return run

                def pv_task(buf, g, c, u, part):
                    def run():
                        n0 = c * CW + part * cw
                        p = lax.dot_general(p_s[g, :, n0:n0 + cw], buf[u * 128:(u + 1) * 128, part * cw:(part + 1) * cw],
                                            _NT, preferred_element_type=_F32)
                        st["o"] = p if part == 0 else st["o"] + p
                        if part == sub - 1:
                            j = g * NU + u
                            o_s[j] = st["o"] if c == 0 else o_s[j] + st["o"]
                    return run

                def out_prep(g):
                    def run():
                        o = jnp.zeros((16, 128), _F32)
                        for u in range(NU):
                            j = g * NU + u
                            r = jnp.sum(jnp.where(head_mask(j), o_s[j], 0.0), axis=0, keepdims=True)
                            o = jnp.where(_iota((16, 128), 0) == u, r, o)
                        st["o5"] = spread5(o.astype(_BF16))
                    return run

                def out_task(g, u):
                    def run():
                        p = tile_dot(diag5(st["o5"][u:u + 1, :]), wo_b, (g * NU + u) * D)
                        st["a"] = st["a"] + p if "a" in st else p
                    return run

                for n, (m, g, c) in enumerate(kv_order):
                    last = n + 1 == len(kv_order)
                    wait(2 + n, LATE if not last or tail_late is None else tail_late)
                    task = (qk_task, pv_task)[m]
                    tasks = [task(kv_b.at[n % 3], g, c, u, part) for u in range(NU) for part in range(sub)]
                    if c == NQ - 1:
                        tasks += [softmax(g)] if m == 0 else [out_prep(g)] + [out_task(g, u) for u in range(NU)]
                    run_tasks(tasks, end[3 + n] + SH + LATE if not last else N + SH)

                j0 = 0
                for t, nj in enumerate(tail[:-1]):
                    wait(T0 + t)
                    if not nocompute:
                        for j in range(j0, j0 + nj):
                            p = jnp.dot(h_s[j], w2_b[j], preferred_element_type=_F32)
                            st["b"] = st["b"] + p if "b" in st else p
                    j0 += nj
                assert tail[-1] == 1 and j0 == F // 128 - 1
                if not nocompute:
                    omg = 1.0 - st["gate"]
                    part = st["gate"] * st["a"] + omg * st["b"]
                    part = jnp.concatenate([part[c:c + 1, :] for c in range(D // 128)], axis=1)
                wait(T0 + len(tail) - 1)
                if not nocompute:
                    w = w2_b[j0].astype(_F32)
                    cols = []
                    for c in range(D // 128):
                        terms = [w[(5 * tr + c) * 8:(5 * tr + c + 1) * 8] * hc_s[tr * 8:(tr + 1) * 8, :] for tr in range(16)]
                        while len(terms) > 1:
                            terms = [a + b for a, b in zip(terms[0::2], terms[1::2])]
                        cols.append(jnp.sum(terms[0], axis=0, keepdims=True))
                    out_b[0] = (part + omg * jnp.concatenate(cols, axis=1)).astype(out_b.dtype)
                else:
                    out_b[...] = jnp.zeros_like(out_b)
                pltpu.make_async_copy(out_b, o_ref, osem).start()

            pl.run_scoped(body, pltpu.SemaphoreType.DMA((2 + len(tail),)))
            pltpu.make_async_copy(out_b, o_ref, osem).wait()

        hbm = pl.BlockSpec(memory_space=pl.ANY)
        return pl.pallas_call(
            kernel,
            out_shape=jax.ShapeDtypeStruct((B, Sq, D), A_x.dtype),
            in_specs=[hbm] * 9,
            out_specs=hbm,
            scratch_shapes=[
                pltpu.VMEM((3, GR, CW), _BF16),
                pltpu.VMEM(wq.shape, _BF16),
                pltpu.VMEM(wo.shape, _BF16),
                pltpu.VMEM(w1.shape, _BF16),
                pltpu.VMEM(w3.shape, _BF16),
                pltpu.VMEM(w2.shape, _BF16),
                pltpu.VMEM((1, 1, D), _BF16),
                pltpu.VMEM((D,), _BF16),
                pltpu.VMEM((D // 8, 128), _F32),
                pltpu.VMEM((D // 32, 16, 384), _BF16),
                pltpu.VMEM((NG * NU, 8, 128), _BF16),
                pltpu.VMEM((NG, 8, W), _F32),
                pltpu.VMEM((NG, 8, W), _BF16),
                pltpu.VMEM((NG * NU, 8, 128), _F32),
                pltpu.VMEM((F // 128, 8, D), _BF16),
                pltpu.VMEM((128, 128), _F32),
                pltpu.VMEM((B, Sq, D), A_x.dtype),
                pltpu.SemaphoreType.DMA(()),
            ],
            compiler_params=pltpu.CompilerParams(vmem_limit_bytes=48 * 1024 * 1024, disable_bounds_checks=nobc),
        )(A_x, kT, vT, wq, wo, w1, w3, w2, gate_w)
    return fn


@jax.jit
def pallas_gated_mix__sliding_block_cached__glu_gated_swiglu__decode_kernel(A_x, A_k_cache, A_v_cache, A_wq, A_wo, B_x, B_w1, B_w3, B_w2, gate_w):
    return make(nobc=False)(A_x, A_k_cache, A_v_cache, A_wq, A_wo, B_x, B_w1, B_w3, B_w2, gate_w)
```

```python
import jax
import jax.numpy as jnp
from jax import lax
import jax.experimental.pallas as pl
import jax.experimental.pallas.tpu as pltpu

_NT = (((1,), (1,)), ((), ()))
_F32 = jnp.float32
_BF16 = jnp.bfloat16

_COLS = 1024
_RUN = 64
_PITCH = 32
_LEAD = 25
_LATE = 11
_SLOTS = 3
_PARTS = 2
_LAST = (6, 4, 2)
_TAIL = (48, 32, 12, 4)


def _tiles(w, n):
    R, C = w.shape
    return w.reshape(R // 8, 8, C // 128, 128).transpose(0, 2, 1, 3).reshape(n, -1, 128)


def _iota(shape, axis):
    return lax.broadcasted_iota(jnp.int32, shape, axis)


def _dot(a, b):
    return jnp.dot(a, b, preferred_element_type=_F32)


def _dot_tiles(lhs, buf, r0):
    acc, n, per = None, lhs.shape[1], buf.shape[1]
    k = 0
    while k < n:
        i, r = divmod(r0 + k, per)
        m = min(n - k, per - r)
        p = _dot(lhs[:, k:k + m], buf[i, r:r + m, :])
        acc = p if acc is None else acc + p
        k += m
    return acc


def _diag(v, rows, period):
    shape = (rows, v.shape[1])
    return jnp.where((_iota(shape, 1) // 8) % period == _iota(shape, 0), v, 0.0).astype(_BF16)


def _repeat8(v, times):
    shape = (128, 128 * times)
    lane = _iota(shape, 1)
    pick = _iota(shape, 0) == 8 * (lane // (8 * times)) + lane % 8
    return _dot(v, jnp.where(pick, 1.0, 0.0).astype(_BF16))


class _Stream:
    def __init__(self):
        self.filled = []
        self.after = []
        self.end = []
        self.slow = []
        self.fast = []
        self.pos = self.nfast = 0
        self.consumed = set()
        self.sems = None

    def group(self, filled, after=None):
        self.filled.append(filled)
        self.after.append(after)
        self.end.append(0)
        return len(self.end) - 1

    def add(self, g, src, dst, fast):
        if fast:
            self.fast.append((len(self.slow), g, src, dst))
        else:
            self.slow.append((g, src, dst))
        self.end[g] = len(self.slow)

    def _start(self, g, src, dst, priority):
        assert self.after[g] is None or self.after[g] in self.consumed
        pltpu.make_async_copy(src, dst, self.sems.at[g]).start(priority=priority)

    def _advance(self, pos):
        while self.pos < pos:
            while self.nfast < len(self.fast) and self.fast[self.nfast][0] + _LEAD <= self.pos:
                self._start(*self.fast[self.nfast][1:], 0)
                self.nfast += 1
            if self.pos < len(self.slow):
                self._start(*self.slow[self.pos], 1)
            self.pos += 1

    def _due(self, groups):
        return min(max(self.end[g] for g in groups) + _LATE, len(self.slow) + 1) + _LEAD

    def stage(self, groups, tasks, then):
        self._advance(self._due(groups))
        for g in groups:
            pltpu.make_async_copy(self.filled[g], self.filled[g], self.sems.at[g]).wait()
        pos0, pos1 = self.pos, self._due(then)
        for k, task in enumerate(tasks):
            task()
            self._advance(pos0 + (pos1 - pos0) * (k + 1) // len(tasks))
        self.consumed.update(groups)


@jax.jit
def pallas_gated_mix__sliding_block_cached__glu_gated_swiglu__decode_kernel(
    A_x: jax.Array,
    A_k_cache: jax.Array,
    A_v_cache: jax.Array,
    A_wq: jax.Array,
    A_wo: jax.Array,
    B_x: jax.Array,
    B_w1: jax.Array,
    B_w3: jax.Array,
    B_w2: jax.Array,
    gate_w: jax.Array,
):
    del B_x
    B, Sq, D = A_x.shape
    _, H, SK, DH = A_k_cache.shape
    F = B_w1.shape[1]
    W = min(4096, max(256, SK // 4))
    scale = DH ** -0.5
    GR = 8 * DH
    NG, NC, NU = H // 8, W // _COLS, GR // 128
    TD, TF, TQ = D // 128, F // 128, H * DH // 128
    NTAIL = sum(_TAIL)
    R2 = (F // 8 - NTAIL) * 8 * TD
    assert B == 1 and Sq == 1 and A_wq.shape[1] == H * DH and sum(_LAST) == NU
    assert H % 8 == 0 and GR % 128 == 0 and W % _COLS == 0 and D % 128 == 0
    assert TD <= 8 and NU <= 16 and TF == 12 and TQ == 48 and NTAIL % 16 == 0 and R2 % _RUN == 0

    def kernel(x_ref, k_ref, v_ref, wq_ref, wo_ref, w1_ref, w3_ref, w2_ref, gw_ref, o_ref,
               kv_b, wq_b, wo_b, w1_b, w3_b, w2_b, x_b, gw_b, out_b,
               x8_s, q_s, s_s, p_s, o_s, h_s):
        stream = _Stream()

        def add_slabs(g, src, dst, u):
            for r in range(0, src.shape[0], 4):
                for (r0, n) in ((r, 1), (r + 1, min(3, src.shape[0] - r - 1))):
                    idx = (pl.ds(r0, n), pl.ds(u * _RUN, _RUN))
                    stream.add(g, src.at[idx], dst.at[idx], r0 == r)

        def add_runs(g, src, dst, u, rows):
            for k, r in enumerate(range(u % _PITCH * _RUN, rows, _PITCH * _RUN)):
                idx = (slice(None), pl.ds(r, _RUN))
                stream.add(g, src.at[idx], dst.at[idx], k == 0)

        g_x, g_gw, g_wq, g_wo, g_w1, g_w3, g_w2 = (
            stream.group(b) for b in (x_b, gw_b, wq_b, wo_b, w1_b, w3_b, w2_b.at[:, pl.ds(0, R2)]))
        stream.add(g_x, x_ref, x_b, True)
        stream.add(g_gw, gw_ref, gw_b, True)
        for u in range(_PITCH):
            add_slabs(g_wq, wq_ref, wq_b, u)
        RF = w1_ref.shape[1]
        for u in range(_PITCH):
            add_runs(g_w2, w2_ref, w2_b, u + 3 * RF // _RUN, R2)
            add_runs(g_w3, w3_ref, w3_b, u + 2 * RF // _RUN, RF)
            add_runs(g_w1, w1_ref, w1_b, u + RF // _RUN, RF)
            add_slabs(g_wo, wo_ref, wo_b, u)

        blocks = [(src, c, hs) for src in (k_ref, v_ref) for c in range(NC) for hs in range(NG)]
        kv_groups = []
        for n, (src, c, hs) in enumerate(blocks):
            buf = kv_b.at[n % _SLOTS]
            u0 = 0
            for nu in (_LAST if n + 1 == len(blocks) else (NU,)):
                g = stream.group(buf.at[pl.ds(u0 * 128, nu * 128)],
                                 kv_groups[n - _SLOTS][0] if n >= _SLOTS else None)
                for r in range(u0 * 128, (u0 + nu) * 128, 32):
                    for (r0, nr) in ((r, 8), (r + 8, 24)):
                        stream.add(g, src.at[pl.ds(hs * GR + r0, nr), pl.ds(SK - W + c * _COLS, _COLS)],
                                   buf.at[pl.ds(r0, nr)], r0 == r)
                kv_groups.append((g, src is v_ref, c, hs, buf, range(u0, u0 + nu)))
                u0 += nu

        tail_groups = []
        t0 = 0
        for nt in _TAIL:
            idx = (slice(None), pl.ds(R2 + t0 * 8 * TD, nt * 8 * TD))
            g = stream.group(w2_b.at[idx])
            stream.add(g, w2_ref.at[idx], w2_b.at[idx], False)
            tail_groups.append((g, t0, nt))
            t0 += nt

        val = {}

        def accumulate(key, p):
            val[key] = val[key] + p if key in val else p

        def own_head(u):
            d = _iota((8, 128), 1) + u * 128 - _iota((8, 128), 0) * DH
            return (d >= 0) & (d < DH)

        def prepare():
            x = x_b[0].astype(_F32)
            gw = gw_b[...].reshape(1, D).astype(_F32)
            val["gate"] = jax.nn.sigmoid(jnp.sum(x * gw, axis=-1, keepdims=True))
            pick = _iota((D, 128), 0) % 8 == _iota((D, 128), 1) % 8
            x8_s[...] = _dot(_diag(x, D // 8, D // 8), jnp.where(pick, 1.0, 0.0).astype(_BF16))

        def project_q(t):
            lhs = _diag(x8_s[t:t + 1, :], 16, 16)
            for b in range(TQ // 16):
                accumulate(("q", b), _dot_tiles(lhs, wq_b, (t * TQ + b * 16) * 8))

        def split_q(j):
            row = val["q", j // 16][j % 16:j % 16 + 1, :]
            q_s[j] = jnp.where(own_head(j % NU), row, 0.0).astype(_BF16)

        def project_ffn(m):
            v = None
            for i in range(4):
                r = jnp.concatenate([x8_s[4 * m + i:4 * m + i + 1, :]] * 3, axis=1)
                v = r if v is None else jnp.where(_iota(r.shape, 1) >= 8 * TF * i, r, v)
            lhs = _diag(v, 16, TF)
            accumulate("w1", _dot_tiles(lhs, w1_b, m * 32 * TF))
            accumulate("w3", _dot_tiles(lhs, w3_b, m * 32 * TF))

        def glu():
            h = (val["w1"] * jax.nn.sigmoid(val["w1"]) * val["w3"]).astype(_BF16)
            val["h"] = _repeat8(h, TD)
            for k, j in enumerate(range(R2 // D, TF)):
                row = h[j:j + 1, :].astype(_F32) * (1.0 - val["gate"])
                h_s[k * 128:(k + 1) * 128, :] = jnp.transpose(jnp.broadcast_to(row, (128, 128)))

        def project_down(j):
            accumulate("ffn", _dot_tiles(_diag(val["h"][j:j + 1, :], 8, TD), w2_b, j * D))

        cw = _COLS // _PARTS

        def scores(buf, c, hs, u, part):
            accumulate(("s", part), _dot(q_s[hs * NU + u],
                                         buf[u * 128:(u + 1) * 128, part * cw:(part + 1) * cw]))
            if u == NU - 1:
                n0 = c * _COLS + part * cw
                s_s[hs, :, n0:n0 + cw] = val.pop(("s", part)) * scale

        def softmax(hs):
            s = s_s[hs]
            e = jnp.exp(s - jnp.max(s, axis=-1, keepdims=True))
            p_s[hs] = (e * (1.0 / jnp.sum(e, axis=-1, keepdims=True))).astype(_BF16)

        def attend(buf, c, hs, u, part):
            n0 = c * _COLS + part * cw
            accumulate("o", lax.dot_general(
                p_s[hs, :, n0:n0 + cw], buf[u * 128:(u + 1) * 128, part * cw:(part + 1) * cw],
                _NT, preferred_element_type=_F32))
            if part == _PARTS - 1:
                j = hs * NU + u
                o_s[j] = val.pop("o") if c == 0 else o_s[j] + val.pop("o")

        def merge_heads(hs, us):
            o = jnp.zeros((16, 128), _F32)
            for u in us:
                row = jnp.sum(jnp.where(own_head(u), o_s[hs * NU + u], 0.0), axis=0, keepdims=True)
                o = jnp.where(_iota((16, 128), 0) == u, row, o)
            val["heads"] = _repeat8(o.astype(_BF16), TD)

        def project_out(hs, u):
            accumulate("attn", _dot_tiles(_diag(val["heads"][u:u + 1, :], 8, TD), wo_b,
                                          (hs * NU + u) * D))

        def mix():
            y = val["gate"] * val["attn"] + (1.0 - val["gate"]) * val["ffn"]
            for c in range(TD):
                val["y", c] = jnp.where(_iota((8, 128), 0) == c, y, 0.0)

        def finish_down(t0, nt):
            for i in range(TD * t0, TD * (t0 + nt), 2):
                w = w2_b[0, R2 + 8 * i:R2 + 8 * i + 16, :].astype(_F32)
                for k in (i, i + 1):
                    t = k // TD
                    accumulate(("y", k % TD), w[8 * (k - i):8 * (k - i) + 8] * h_s[8 * t:8 * t + 8, :])

        def task(f, *args):
            return lambda: f(*args)

        stages = [
            ([g_x, g_gw, g_wq],
             [prepare] + [task(project_q, t) for t in range(D // 8)]
             + [task(split_q, j) for j in range(TQ)]),
            ([g_wo, g_w1, g_w3, g_w2],
             [task(project_ffn, m) for m in range(D // 32)] + [glu]
             + [task(project_down, j) for j in range(R2 // D)]),
        ]
        for (g, is_v, c, hs, buf, us) in kv_groups:
            tasks = [task(attend if is_v else scores, buf, c, hs, u, part)
                     for u in us for part in range(_PARTS)]
            if c == NC - 1 and is_v:
                tasks += [task(merge_heads, hs, us)] + [task(project_out, hs, u) for u in us]
            elif c == NC - 1:
                tasks += [task(softmax, hs)]
            stages.append(([g], tasks))
        stages[-1][1].append(mix)
        stages += [([g], [task(finish_down, t0, nt)]) for (g, t0, nt) in tail_groups]

        def run(sems, out_sem):
            stream.sems = sems
            for (groups, tasks), (then, _) in zip(stages, stages[1:] + stages[-1:]):
                stream.stage(groups, tasks, then)
            assert len(stream.consumed) == len(stream.filled) and stream.nfast == len(stream.fast)
            out_b[0] = jnp.concatenate(
                [jnp.sum(val["y", c], axis=0, keepdims=True) for c in range(TD)],
                axis=1).astype(out_b.dtype)
            store = pltpu.make_async_copy(out_b, o_ref, out_sem)
            store.start()
            store.wait()

        pl.run_scoped(run, pltpu.SemaphoreType.DMA((len(stream.filled),)), pltpu.SemaphoreType.DMA(()))

    kT = jnp.swapaxes(A_k_cache, 2, 3).reshape(H * DH, SK)
    vT = jnp.swapaxes(A_v_cache, 2, 3).reshape(H * DH, SK)
    slabs = D * TQ // (_PITCH * _RUN)
    weights = [_tiles(A_wq, slabs), _tiles(A_wo, slabs), _tiles(B_w1, 1), _tiles(B_w3, 1), _tiles(B_w2, 1)]
    hbm = pl.BlockSpec(memory_space=pl.ANY)
    return pl.pallas_call(
        kernel,
        out_shape=jax.ShapeDtypeStruct((B, Sq, D), A_x.dtype),
        in_specs=[hbm] * 9,
        out_specs=hbm,
        scratch_shapes=[
            pltpu.VMEM((_SLOTS, GR, _COLS), _BF16),
            *[pltpu.VMEM(w.shape, _BF16) for w in weights],
            pltpu.VMEM(A_x.shape, _BF16),
            pltpu.VMEM(gate_w.shape, _BF16),
            pltpu.VMEM((B, Sq, D), A_x.dtype),
            pltpu.VMEM((D // 8, 128), _F32),
            pltpu.VMEM((TQ, 8, 128), _BF16),
            pltpu.VMEM((NG, 8, W), _F32),
            pltpu.VMEM((NG, 8, W), _BF16),
            pltpu.VMEM((TQ, 8, 128), _F32),
            pltpu.VMEM((NTAIL * 8, 128), _F32),
        ],
        compiler_params=pltpu.CompilerParams(vmem_limit_bytes=48 * 1024 * 1024),
    )(A_x, kT, vT, *weights, gate_w)
```

```python
import jax
import jax.numpy as jnp
from jax import lax
import jax.experimental.pallas as pl
import jax.experimental.pallas.tpu as pltpu

_NT = (((1,), (1,)), ((), ()))
_F32 = jnp.float32
_BF16 = jnp.bfloat16

_COLS = 1024
_RUN = 64
_PITCH = 32
_LEAD = 25
_RAMP = 8
_LATE = 11
_SLOTS = 3
_PARTS = 2
_LAST = (5, 4, 3)
_TAIL = (48, 16, 10, 4, 2)


def _tiles(w, n):
    R, C = w.shape
    return w.reshape(R // 8, 8, C // 128, 128).transpose(0, 2, 1, 3).reshape(n, -1, 128)


def _iota(shape, axis):
    return lax.broadcasted_iota(jnp.int32, shape, axis)


def _dot(a, b):
    return jnp.dot(a, b, preferred_element_type=_F32)


def _dot_tiles(lhs, buf, r0):
    acc, n, per = None, lhs.shape[1], buf.shape[1]
    k = 0
    while k < n:
        i, r = divmod(r0 + k, per)
        m = min(n - k, per - r)
        p = _dot(lhs[:, k:k + m], buf[i, r:r + m, :])
        acc = p if acc is None else acc + p
        k += m
    return acc


def _diag(v, rows, period):
    shape = (rows, v.shape[1])
    return jnp.where((_iota(shape, 1) // 8) % period == _iota(shape, 0), v, 0.0).astype(_BF16)


def _repeat8(v, times):
    shape = (128, 128 * times)
    lane = _iota(shape, 1)
    pick = _iota(shape, 0) == 8 * (lane // (8 * times)) + lane % 8
    return _dot(v, jnp.where(pick, 1.0, 0.0).astype(_BF16))


class _Stream:
    def __init__(self):
        self.filled = []
        self.after = []
        self.end = []
        self.slow = []
        self.fast = []
        self.pos = self.nfast = 0
        self.consumed = set()
        self.sems = None

    def group(self, filled, after=None):
        self.filled.append(filled)
        self.after.append(after)
        self.end.append(0)
        return len(self.end) - 1

    def add(self, g, src, dst, fast):
        if fast:
            place = len(self.slow)
            self.fast.append((min(place + _LEAD, place * _RAMP), g, src, dst))
        else:
            self.slow.append((g, src, dst))
        self.end[g] = len(self.slow)

    def _start(self, g, src, dst, priority):
        assert self.after[g] is None or self.after[g] in self.consumed
        pltpu.make_async_copy(src, dst, self.sems.at[g]).start(priority=priority)

    def _advance(self, pos):
        while self.pos < pos:
            while self.nfast < len(self.fast) and self.fast[self.nfast][0] <= self.pos:
                self._start(*self.fast[self.nfast][1:], 0)
                self.nfast += 1
            if self.pos < len(self.slow):
                self._start(*self.slow[self.pos], 1)
            self.pos += 1

    def _due(self, groups):
        return min(max(self.end[g] for g in groups) + _LATE, len(self.slow) + 1) + _LEAD

    def stage(self, groups, tasks, then):
        self._advance(self._due(groups))
        for g in groups:
            pltpu.make_async_copy(self.filled[g], self.filled[g], self.sems.at[g]).wait()
        pos0, pos1 = self.pos, self._due(then)
        for k, task in enumerate(tasks):
            task()
            self._advance(pos0 + (pos1 - pos0) * (k + 1) // len(tasks))
        self.consumed.update(groups)


@jax.jit
def pallas_gated_mix__sliding_block_cached__glu_gated_swiglu__decode_kernel(
    A_x: jax.Array,
    A_k_cache: jax.Array,
    A_v_cache: jax.Array,
    A_wq: jax.Array,
    A_wo: jax.Array,
    B_x: jax.Array,
    B_w1: jax.Array,
    B_w3: jax.Array,
    B_w2: jax.Array,
    gate_w: jax.Array,
):
    del B_x
    B, Sq, D = A_x.shape
    _, H, SK, DH = A_k_cache.shape
    F = B_w1.shape[1]
    W = min(4096, max(256, SK // 4))
    scale = DH ** -0.5
    GR = 8 * DH
    NG, NC, NU = H // 8, W // _COLS, GR // 128
    TD, TF, TQ = D // 128, F // 128, H * DH // 128
    NTAIL = sum(_TAIL)
    R2 = (F // 8 - NTAIL) * 8 * TD
    assert B == 1 and Sq == 1 and A_wq.shape[1] == H * DH and sum(_LAST) == NU
    assert H % 8 == 0 and GR % 128 == 0 and W % _COLS == 0 and D % 128 == 0
    assert TD <= 8 and NU <= 16 and TF == 12 and TQ == 48 and NTAIL % 16 == 0 and R2 % _RUN == 0

    def kernel(x_ref, k_ref, v_ref, wq_ref, wo_ref, w1_ref, w3_ref, w2_ref, gw_ref, o_ref,
               kv_b, wq_b, wo_b, w1_b, w3_b, w2_b, x_b, gw_b, out_b,
               x8_s, q_s, s_s, p_s, o_s, h_s):
        stream = _Stream()

        def add_slabs(g, src, dst, u):
            for r in range(0, src.shape[0], 4):
                for (r0, n) in ((r, 1), (r + 1, min(3, src.shape[0] - r - 1))):
                    idx = (pl.ds(r0, n), pl.ds(u * _RUN, _RUN))
                    stream.add(g, src.at[idx], dst.at[idx], r0 == r)

        def add_runs(g, src, dst, u, rows):
            for k, r in enumerate(range(u % _PITCH * _RUN, rows, _PITCH * _RUN)):
                idx = (slice(None), pl.ds(r, _RUN))
                stream.add(g, src.at[idx], dst.at[idx], k == 0)

        g_x, g_gw, g_wq, g_wo, g_w1, g_w3, g_w2 = (
            stream.group(b) for b in (x_b, gw_b, wq_b, wo_b, w1_b, w3_b, w2_b.at[:, pl.ds(0, R2)]))
        for u in range(_PITCH):
            add_slabs(g_wq, wq_ref, wq_b, u)
        stream.add(g_x, x_ref, x_b, True)
        stream.add(g_gw, gw_ref, gw_b, True)
        RF = w1_ref.shape[1]
        for u in range(_PITCH):
            add_runs(g_w2, w2_ref, w2_b, u + 3 * RF // _RUN, R2)
            add_runs(g_w3, w3_ref, w3_b, u + 2 * RF // _RUN, RF)
            add_runs(g_w1, w1_ref, w1_b, u + RF // _RUN, RF)
            add_slabs(g_wo, wo_ref, wo_b, u)

        blocks = [(src, c, hs) for src in (k_ref, v_ref) for c in range(NC) for hs in range(NG)]
        kv_groups = []
        for n, (src, c, hs) in enumerate(blocks):
            buf = kv_b.at[n % _SLOTS]
            u0 = 0
            for nu in (_LAST if n + 1 == len(blocks) else (NU,)):
                g = stream.group(buf.at[pl.ds(u0 * 128, nu * 128)],
                                 kv_groups[n - _SLOTS][0] if n >= _SLOTS else None)
                for r in range(u0 * 128, (u0 + nu) * 128, 32):
                    for (r0, nr) in ((r, 8), (r + 8, 24)):
                        stream.add(g, src.at[pl.ds(hs * GR + r0, nr), pl.ds(SK - W + c * _COLS, _COLS)],
                                   buf.at[pl.ds(r0, nr)], r0 == r)
                kv_groups.append((g, src is v_ref, c, hs, buf, range(u0, u0 + nu)))
                u0 += nu

        tail_groups = []
        t0 = 0
        for nt in _TAIL:
            g = stream.group(w2_b.at[:, pl.ds(R2 + t0 * 8 * TD, nt * 8 * TD)])
            for t in range(t0, t0 + nt, 4):
                idx = (slice(None), pl.ds(R2 + t * 8 * TD, min(4, t0 + nt - t) * 8 * TD))
                stream.add(g, w2_ref.at[idx], w2_b.at[idx], False)
            tail_groups.append((g, t0, nt))
            t0 += nt

        val = {}

        def accumulate(key, p):
            val[key] = val[key] + p if key in val else p

        def own_head(u):
            d = _iota((8, 128), 1) + u * 128 - _iota((8, 128), 0) * DH
            return (d >= 0) & (d < DH)

        def prepare():
            x = x_b[0].astype(_F32)
            gw = gw_b[...].reshape(1, D).astype(_F32)
            val["gate"] = jax.nn.sigmoid(jnp.sum(x * gw, axis=-1, keepdims=True))
            pick = _iota((D, 128), 0) % 8 == _iota((D, 128), 1) % 8
            x8_s[...] = _dot(_diag(x, D // 8, D // 8), jnp.where(pick, 1.0, 0.0).astype(_BF16))

        def project_q(t):
            lhs = _diag(x8_s[t:t + 1, :], 16, 16)
            for b in range(TQ // 16):
                accumulate(("q", b), _dot_tiles(lhs, wq_b, (t * TQ + b * 16) * 8))

        def split_q(j):
            row = val["q", j // 16][j % 16:j % 16 + 1, :]
            q_s[j] = jnp.where(own_head(j % NU), row, 0.0).astype(_BF16)

        def project_ffn(m):
            v = None
            for i in range(4):
                r = jnp.concatenate([x8_s[4 * m + i:4 * m + i + 1, :]] * 3, axis=1)
                v = r if v is None else jnp.where(_iota(r.shape, 1) >= 8 * TF * i, r, v)
            lhs = _diag(v, 16, TF)
            accumulate("w1", _dot_tiles(lhs, w1_b, m * 32 * TF))
            accumulate("w3", _dot_tiles(lhs, w3_b, m * 32 * TF))

        def glu():
            h = (val["w1"] * jax.nn.sigmoid(val["w1"]) * val["w3"]).astype(_BF16)
            val["h"] = _repeat8(h, TD)
            for k, j in enumerate(range(R2 // D, TF)):
                row = h[j:j + 1, :].astype(_F32) * (1.0 - val["gate"])
                h_s[k * 128:(k + 1) * 128, :] = jnp.transpose(jnp.broadcast_to(row, (128, 128)))

        def project_down(j):
            accumulate("ffn", _dot_tiles(_diag(val["h"][j:j + 1, :], 8, TD), w2_b, j * D))

        cw = _COLS // _PARTS

        def scores(buf, c, hs, u, part):
            accumulate(("s", part), _dot(q_s[hs * NU + u],
                                         buf[u * 128:(u + 1) * 128, part * cw:(part + 1) * cw]))
            if u == NU - 1:
                n0 = c * _COLS + part * cw
                s_s[hs, :, n0:n0 + cw] = val.pop(("s", part)) * scale

        def softmax(hs):
            s = s_s[hs]
            e = jnp.exp(s - jnp.max(s, axis=-1, keepdims=True))
            p_s[hs] = (e * (1.0 / jnp.sum(e, axis=-1, keepdims=True))).astype(_BF16)

        def attend(buf, c, hs, u, part):
            n0 = c * _COLS + part * cw
            accumulate("o", lax.dot_general(
                p_s[hs, :, n0:n0 + cw], buf[u * 128:(u + 1) * 128, part * cw:(part + 1) * cw],
                _NT, preferred_element_type=_F32))
            if part == _PARTS - 1:
                j = hs * NU + u
                o_s[j] = val.pop("o") if c == 0 else o_s[j] + val.pop("o")

        def merge_heads(hs, us):
            o = jnp.zeros((16, 128), _F32)
            for u in us:
                row = jnp.sum(jnp.where(own_head(u), o_s[hs * NU + u], 0.0), axis=0, keepdims=True)
                o = jnp.where(_iota((16, 128), 0) == u, row, o)
            val["heads"] = _repeat8(o.astype(_BF16), TD)

        def project_out(hs, u):
            accumulate("attn", _dot_tiles(_diag(val["heads"][u:u + 1, :], 8, TD), wo_b,
                                          (hs * NU + u) * D))

        def mix():
            y = val["gate"] * val["attn"] + (1.0 - val["gate"]) * val["ffn"]
            for c in range(TD):
                val["y", c] = jnp.where(_iota((8, 128), 0) == c, y, 0.0)

        def finish_down(t0, nt):
            for i in range(TD * t0, TD * (t0 + nt), 2):
                w = w2_b[0, R2 + 8 * i:R2 + 8 * i + 16, :].astype(_F32)
                for k in (i, i + 1):
                    t = k // TD
                    accumulate(("y", k % TD), w[8 * (k - i):8 * (k - i) + 8] * h_s[8 * t:8 * t + 8, :])

        def task(f, *args):
            return lambda: f(*args)

        stages = [
            ([g_x, g_gw, g_wq],
             [prepare] + [task(project_q, t) for t in range(D // 8)]
             + [task(split_q, j) for j in range(TQ)]),
            ([g_wo, g_w1, g_w3, g_w2],
             [task(project_ffn, m) for m in range(D // 32)] + [glu]
             + [task(project_down, j) for j in range(R2 // D)]),
        ]
        for (g, is_v, c, hs, buf, us) in kv_groups:
            tasks = [task(attend if is_v else scores, buf, c, hs, u, part)
                     for u in us for part in range(_PARTS)]
            if c == NC - 1 and is_v:
                tasks += [task(merge_heads, hs, us)] + [task(project_out, hs, u) for u in us]
            elif c == NC - 1:
                tasks += [task(softmax, hs)]
            stages.append(([g], tasks))
        stages[-1][1].append(mix)
        stages += [([g], [task(finish_down, t0, nt)]) for (g, t0, nt) in tail_groups]

        def run(sems, out_sem):
            stream.sems = sems
            for (groups, tasks), (then, _) in zip(stages, stages[1:] + stages[-1:]):
                stream.stage(groups, tasks, then)
            assert len(stream.consumed) == len(stream.filled) and stream.nfast == len(stream.fast)
            out_b[0] = jnp.concatenate(
                [jnp.sum(val["y", c], axis=0, keepdims=True) for c in range(TD)],
                axis=1).astype(out_b.dtype)
            store = pltpu.make_async_copy(out_b, o_ref, out_sem)
            store.start()
            store.wait()

        pl.run_scoped(run, pltpu.SemaphoreType.DMA((len(stream.filled),)), pltpu.SemaphoreType.DMA(()))

    kT = jnp.swapaxes(A_k_cache, 2, 3).reshape(H * DH, SK)
    vT = jnp.swapaxes(A_v_cache, 2, 3).reshape(H * DH, SK)
    slabs = D * TQ // (_PITCH * _RUN)
    weights = [_tiles(A_wq, slabs), _tiles(A_wo, slabs), _tiles(B_w1, 1), _tiles(B_w3, 1), _tiles(B_w2, 1)]
    hbm = pl.BlockSpec(memory_space=pl.ANY)
    return pl.pallas_call(
        kernel,
        out_shape=jax.ShapeDtypeStruct((B, Sq, D), A_x.dtype),
        in_specs=[hbm] * 9,
        out_specs=hbm,
        scratch_shapes=[
            pltpu.VMEM((_SLOTS, GR, _COLS), _BF16),
            *[pltpu.VMEM(w.shape, _BF16) for w in weights],
            pltpu.VMEM(A_x.shape, _BF16),
            pltpu.VMEM(gate_w.shape, _BF16),
            pltpu.VMEM((B, Sq, D), A_x.dtype),
            pltpu.VMEM((D // 8, 128), _F32),
            pltpu.VMEM((TQ, 8, 128), _BF16),
            pltpu.VMEM((NG, 8, W), _F32),
            pltpu.VMEM((NG, 8, W), _BF16),
            pltpu.VMEM((TQ, 8, 128), _F32),
            pltpu.VMEM((NTAIL * 8, 128), _F32),
        ],
        compiler_params=pltpu.CompilerParams(vmem_limit_bytes=48 * 1024 * 1024),
    )(A_x, kT, vT, *weights, gate_w)
```
